```python
import os as _os
_os.environ.setdefault('JAX_PLATFORMS', 'cpu')
import jax
import jax.numpy as jnp

def _softmax(x, axis=-1):
    return jax.nn.softmax(x, axis=axis)

def _gelu(x):
    return jax.nn.gelu(x, approximate=True)

def _silu(x):
    return jax.nn.silu(x)

def _sigmoid(x):
    return jax.nn.sigmoid(x)

def _layernorm(x, axis=-1, eps=1e-05):
    m = jnp.mean(x, axis=axis, keepdims=True)
    v = jnp.var(x, axis=axis, keepdims=True)
    return (x - m) / jnp.sqrt(v + eps)

def _scatter_add(tgt, idx, src, axis=0):
    return tgt.at[idx].add(src)

def _segment_sum(src, seg, n):
    return jax.ops.segment_sum(src, seg, n)

class _Rng:

    def __init__(self, key):
        self._k = key

    def _next(self):
        self._k, sub = jax.random.split(self._k)
        return sub

    def normal(self, shape):
        return jax.random.normal(self._next(), shape, dtype=jnp.bfloat16)

    def randint(self, lo, hi, shape):
        return jax.random.randint(self._next(), shape, lo, hi, dtype=jnp.int32)

    def uniform(self, shape, lo=0.0, hi=1.0):
        return jax.random.uniform(self._next(), shape, jnp.bfloat16, lo, hi)

    def permutation(self, n):
        return jax.random.permutation(self._next(), n)
kernel_name = 'adaLN_cond__mha_block__dense_activation_squared_relu__prompt'

def setup_inputs():
    _rng = _Rng(jax.random.key(int.from_bytes(__import__("os").urandom(4), "little")))
    _w = lambda a: (lambda t: t.astype(jnp.bfloat16) if jnp.issubdtype(t.dtype, jnp.floating) else t)(jnp.asarray(a))

    def _A_setup():
        B, S, D, H = (1, 2048, 512, 32)
        return {'x': _w((lambda *s: _rng.normal(s) * 0.05)(B, S, D)), 'wqkv': _w((lambda *s: _rng.normal(s) * 0.1)(D, 3 * D)), 'wo': _w((lambda *s: _rng.normal(s) * 0.05)(D, D))}
    _A_in = _A_setup()

    def _B_setup():
        B, S, D, F = (1, 2048, 512, 1792)
        return {'x': _w((lambda *s: _rng.normal(s) * 0.05)(B, S, D)), 'w1': _w((lambda *s: _rng.normal(s) * 0.05)(D, F)), 'b1': _w((lambda *s: _rng.normal(s) * 0.05)(F)), 'w2': _w((lambda *s: _rng.normal(s) * 0.05)(F, D)), 'b2': _w((lambda *s: _rng.normal(s) * 0.05)(D))}
    _B_in = _B_setup()
    return {'A_x': _A_in['x'], 'A_wqkv': _A_in['wqkv'], 'A_wo': _A_in['wo'], 'B_x': _B_in['x'], 'B_w1': _B_in['w1'], 'B_b1': _B_in['b1'], 'B_w2': _B_in['w2'], 'B_b2': _B_in['b2'], 'c': _w((lambda *s: _rng.normal(s) * 0.05)(1, 512) * 8.0), 'w_mod': _w((lambda *s: _rng.normal(s) * 0.05)(512, 6 * 512) * 512 ** (-0.5) * 8.0)}

def reference(A_x, A_wqkv, A_wo, B_x, B_w1, B_b1, B_w2, B_b2, c, w_mod):

    def _A_ref(x, wqkv, wo):
        B, S, D = x.shape
        H = 32
        Dh = D // H
        qkv = (lambda x, *d: x.transpose(*d))((x @ wqkv).reshape(B, S, 3, H, Dh), 2, 0, 3, 1, 4)
        q, k, v = (qkv[0], qkv[1], qkv[2])
        scores = jnp.einsum('bhqd,bhkd->bhqk', q, k) * Dh ** (-0.5)
        p = _softmax(scores, axis=-1)
        o = jnp.einsum('bhqk,bhkd->bhqd', p, v)
        return (lambda x, *d: x.transpose(*d))(o, 0, 2, 1, 3).reshape(B, S, D) @ wo

    def _B_ref(x, w1, b1, w2, b2):
        h = jnp.einsum('bsd,df->bsf', x, w1) + b1
        zero = jnp.zeros_like(h)
        r = jnp.where(h > zero, h, zero)
        h = r * r
        out = jnp.einsum('bsf,fd->bsd', h, w2) + b2
        return out
    x = A_x
    mod = (_silu(c) @ w_mod).reshape(c.shape[0], 6, 1, -1)
    sa, ca, ga, sb, cb, gb = (mod[:, 0].copy(), mod[:, 1].copy(), mod[:, 2].copy(), mod[:, 3].copy(), mod[:, 4].copy(), mod[:, 5].copy())
    h = _layernorm(x, axis=-1) * (1 + ca) + sa
    x = x + ga * _A_ref(h, A_wqkv, A_wo)
    h = _layernorm(x, axis=-1) * (1 + cb) + sb
    x = x + gb * _B_ref(h, B_w1, B_b1, B_w2, B_b2)
    return x
```

```python
import jax
import jax.numpy as jnp
from jax import lax
import jax.experimental.pallas as pl
import jax.experimental.pallas.tpu as pltpu

_D = 512
_H = 32
_DH = 16
_LOG2E = 1.4426950408889634
_EPS = 1e-5
_NT = (((1,), (1,)), ((), ()))
_TN = (((0,), (0,)), ((), ()))


def _ln_mod(x, scale, shift):
    m = jnp.mean(x, axis=-1, keepdims=True)
    xc = x - m
    v = jnp.mean(xc * xc, axis=-1, keepdims=True)
    return xc * lax.rsqrt(v + _EPS) * scale + shift


def _red8(fn, s):
    return fn(s.reshape(s.shape[0] // 8, 8, s.shape[1]), axis=0)


def make_kernel(S, F, tq, ck, U, td, tm, peel):
    nx = S // tm
    nd = S // td
    T = (S // tq) * _H

    def kernel(x_hbm, wqkv_hbm, wo_hbm, w1_hbm, b1_ref, w2_hbm, b2_ref, c_ref, wmod_hbm,
               out_hbm,
               x_ref, wqkv_ref, wo_ref, w1_ref, w2_ref, wmod_ref, out_ref,
               mod_ref, qT_ref, k_ref, vT_ref, oT_ref, s0_ref, s1_ref, m0_ref, m1_ref,
               sem_in, sem_x, sem_out):
        cp_wm0 = pltpu.make_async_copy(wmod_hbm.at[:, 0:2 * _D], wmod_ref.at[:, 0:2 * _D], sem_in.at[0])
        cp_x = [pltpu.make_async_copy(x_hbm.at[t * tm:(t + 1) * tm, :], x_ref.at[t * tm:(t + 1) * tm, :], sem_x.at[t])
                for t in range(nx)]
        cp_wqkv = pltpu.make_async_copy(wqkv_hbm, wqkv_ref, sem_in.at[1])
        cp_wm1 = pltpu.make_async_copy(wmod_hbm.at[:, 2 * _D:6 * _D], wmod_ref.at[:, 2 * _D:6 * _D], sem_in.at[2])
        cp_wo = pltpu.make_async_copy(wo_hbm, wo_ref, sem_in.at[3])
        cp_w1 = pltpu.make_async_copy(w1_hbm, w1_ref, sem_in.at[4])
        cp_w2 = pltpu.make_async_copy(w2_hbm, w2_ref, sem_in.at[5])
        cp_wm0.start()
        cp_wqkv.start()
        for cp in cp_x:
            cp.start()
        cp_wm1.start()
        cp_wo.start()
        cp_w1.start()
        cp_w2.start()

        c = c_ref[...].astype(jnp.float32)
        sc = (c * jax.nn.sigmoid(c)).astype(jnp.bfloat16)
        sc16 = jnp.broadcast_to(sc, (16, _D))
        cp_wm0.wait()
        mod_a = jnp.dot(sc16, wmod_ref[:, 0:2 * _D], preferred_element_type=jnp.float32)[0:1]
        sa = mod_a[:, 0:_D]
        ca1 = 1.0 + mod_a[:, _D:2 * _D]
        cp_wqkv.wait()
        wqT = wqkv_ref[:, 0:_D].astype(jnp.float32).T.astype(jnp.bfloat16)
        wvT = wqkv_ref[:, 2 * _D:3 * _D].astype(jnp.float32).T.astype(jnp.bfloat16)
        wk = wqkv_ref[:, _D:2 * _D]
        for t in range(nx):
            cp_x[t].wait()
            rows = slice(t * tm, (t + 1) * tm)
            x = x_ref[rows, :].astype(jnp.float32)
            h = _ln_mod(x, ca1, sa).astype(jnp.bfloat16)
            qT = lax.dot_general(wqT, h, _NT, preferred_element_type=jnp.float32)
            qT_ref[:, rows] = (qT * (0.25 * _LOG2E)).astype(jnp.bfloat16)
            k = jnp.dot(h, wk, preferred_element_type=jnp.float32).astype(jnp.bfloat16)
            for g in range(4):
                k_ref[g, rows, :] = k[:, g * 128:(g + 1) * 128]
            vT = lax.dot_general(wvT, h, _NT, preferred_element_type=jnp.float32)
            vT_ref[:, rows] = vT.astype(jnp.bfloat16)

        row_head = lax.broadcasted_iota(jnp.int32, (128, tq), 0) // _DH

        def step(tA, sA_ref, mA_ref, tB, sB_ref, mB_ref):
            doA = tA is not None
            doB = tB is not None
            if doA:
                hA = tA % _H
                qa0 = pl.multiple_of((tA // _H) * tq, tq)
                g = hA // 8
                qg = qT_ref[pl.ds(pl.multiple_of(g * 128, 128), 128), pl.ds(qa0, tq)]
                qm = jnp.where(row_head == hA % 8, qg, jnp.zeros_like(qg))
                mx = None
            if doB:
                h0 = pl.multiple_of((tB % _H) * _DH, _DH)
                qb0 = pl.multiple_of((tB // _H) * tq, tq)
                m = jnp.max(mB_ref[...], axis=0, keepdims=True)
                l = None
                acc = None
            for ci in range(S // ck):
                sl = slice(ci * ck, (ci + 1) * ck)
                if doA:
                    s = jnp.dot(k_ref[g, sl, :], qm, preferred_element_type=jnp.float32)
                    sA_ref[sl, :] = s
                    cm = _red8(jnp.max, s)
                    mx = cm if mx is None else jnp.maximum(mx, cm)
                if doB:
                    p = jnp.exp2(sB_ref[sl, :] - m)
                    cl = _red8(jnp.sum, p)
                    l = cl if l is None else l + cl
                    o = jnp.dot(vT_ref[pl.ds(h0, _DH), sl], p.astype(jnp.bfloat16),
                                preferred_element_type=jnp.float32)
                    acc = o if acc is None else acc + o
            if doA:
                mA_ref[...] = mx
            if doB:
                l = jnp.sum(l, axis=0, keepdims=True)
                oT_ref[pl.ds(h0, _DH), pl.ds(qb0, tq)] = (acc * (1.0 / l)).astype(jnp.bfloat16)

        bufs = ((s0_ref, m0_ref), (s1_ref, m1_ref))
        step(0, s0_ref, m0_ref, None, None, None)

        def att_body(it, carry):
            for u in range(U):
                t = it * U + u
                step(jnp.minimum(t + 1, T - 1), *bufs[(u + 1) % 2], t, *bufs[u % 2])
            return carry

        if peel:
            lax.fori_loop(0, T // U - 1, att_body, 0)
            for u in range(U):
                t = T - U + u
                step(t + 1 if u < U - 1 else None, *bufs[(u + 1) % 2], t, *bufs[u % 2])
        else:
            lax.fori_loop(0, T // U, att_body, 0)

        cp_wm1.wait()
        mod_b = jnp.dot(sc16, wmod_ref[:, 2 * _D:6 * _D], preferred_element_type=jnp.float32)[0:1]
        ga = mod_b[:, 0:_D]
        sb = mod_b[:, _D:2 * _D]
        cb1 = 1.0 + mod_b[:, 2 * _D:3 * _D]
        gb = mod_b[:, 3 * _D:4 * _D]
        cp_wo.wait()
        cp_w1.wait()
        cp_w2.wait()
        b1 = b1_ref[...].astype(jnp.float32)
        b2 = b2_ref[...].astype(jnp.float32)
        cp_out = []
        for t in range(nd):
            rows = slice(t * td, (t + 1) * td)
            attn = lax.dot_general(oT_ref[:, rows], wo_ref[...], _TN, preferred_element_type=jnp.float32)
            x1 = x_ref[rows, :].astype(jnp.float32) + ga * attn
            h2 = _ln_mod(x1, cb1, sb).astype(jnp.bfloat16)
            u = jnp.dot(h2, w1_ref[...], preferred_element_type=jnp.float32) + b1
            r = jnp.maximum(u, 0.0)
            r = (r * r).astype(jnp.bfloat16)
            f = jnp.dot(r, w2_ref[...], preferred_element_type=jnp.float32) + b2
            out_ref[rows, :] = (x1 + gb * f).astype(out_ref.dtype)
            cp = pltpu.make_async_copy(out_ref.at[rows, :], out_hbm.at[rows, :], sem_out.at[t])
            cp.start()
            cp_out.append(cp)
        for cp in cp_out:
            cp.wait()

    return kernel


def run(A_x, A_wqkv, A_wo, B_x, B_w1, B_b1, B_w2, B_b2, c, w_mod, *, tq=512, ck=128, U=2, td=512, tm=512,
        peel=False, flags=None):
    B, S, D = A_x.shape
    F = B_w1.shape[1]
    hbm = pl.BlockSpec(memory_space=pl.ANY)
    vmem = pl.BlockSpec(memory_space=pltpu.VMEM)
    bf = jnp.bfloat16
    out = pl.pallas_call(
        make_kernel(S, F, tq, ck, U, td, tm, peel),
        in_specs=[hbm, hbm, hbm, hbm, vmem, hbm, vmem, vmem, hbm],
        out_specs=hbm,
        out_shape=jax.ShapeDtypeStruct((S, D), A_x.dtype),
        scratch_shapes=[
            pltpu.VMEM((S, D), bf), pltpu.VMEM((D, 3 * D), bf), pltpu.VMEM((D, D), bf),
            pltpu.VMEM((D, F), bf), pltpu.VMEM((F, D), bf), pltpu.VMEM((D, 6 * D), bf),
            pltpu.VMEM((S, D), bf),
            pltpu.VMEM((8, 6 * D), jnp.float32),
            pltpu.VMEM((D, S), bf), pltpu.VMEM((4, S, 128), bf), pltpu.VMEM((D, S), bf), pltpu.VMEM((D, S), bf),
            pltpu.VMEM((S, tq), jnp.float32), pltpu.VMEM((S, tq), jnp.float32),
            pltpu.VMEM((8, tq), jnp.float32), pltpu.VMEM((8, tq), jnp.float32),
            pltpu.SemaphoreType.DMA((6,)), pltpu.SemaphoreType.DMA((S // tm,)), pltpu.SemaphoreType.DMA((S // td,)),
        ],
        compiler_params=pltpu.CompilerParams(vmem_limit_bytes=100 * 1024 * 1024, flags=flags),
    )(A_x.reshape(S, D), A_wqkv, A_wo, B_w1, B_b1.reshape(1, F), B_w2, B_b2.reshape(1, D), c, w_mod)
    return out.reshape(B, S, D)


@jax.jit
def pallas_adaLN_cond__mha_block__dense_activation_squared_relu__prompt_kernel(
    A_x: jax.Array,
    A_wqkv: jax.Array,
    A_wo: jax.Array,
    B_x: jax.Array,
    B_w1: jax.Array,
    B_b1: jax.Array,
    B_w2: jax.Array,
    B_b2: jax.Array,
    c: jax.Array,
    w_mod: jax.Array,
):
    return run(A_x, A_wqkv, A_wo, B_x, B_w1, B_b1, B_w2, B_b2, c, w_mod, tq=256, ck=128)
```

```python
import jax
import jax.numpy as jnp
from jax import lax
import jax.experimental.pallas as pl
import jax.experimental.pallas.tpu as pltpu

_D = 512
_H = 32
_DH = 16
_LOG2E = 1.4426950408889634
_EPS = 1e-5
_NT = (((1,), (1,)), ((), ()))
_TN = (((0,), (0,)), ((), ()))


def _ln_mod(x, scale, shift):
    m = jnp.mean(x, axis=-1, keepdims=True)
    xc = x - m
    v = jnp.mean(xc * xc, axis=-1, keepdims=True)
    return xc * lax.rsqrt(v + _EPS) * scale + shift


def _red8(fn, s):
    return fn(s.reshape(s.shape[0] // 8, 8, s.shape[1]), axis=0)


def _pk(v):
    return pltpu.bitcast(v, jnp.uint32)


def _upk(v):
    return pltpu.bitcast(v, jnp.bfloat16)


def _st_blocks(ref, b0, val):
    for i in range(val.shape[1] // 128):
        ref[b0 + i] = _pk(val[:, i * 128:(i + 1) * 128])


def make_kernel(S, F, tq, ck, ca, U, td, tm, DL, var):
    nx = S // tm
    nd = S // td
    T = (S // tq) * _H

    def kernel(x_hbm, wqkv_hbm, wo_hbm, w1_hbm, b1_ref, w2_hbm, b2_ref, c_ref, wmod_hbm,
               out_hbm,
               x_ref, wqkv_ref, wo_ref, w1_ref, w2_ref, wmod_ref, out_ref,
               qT_ref, k_ref, vT_ref, oT_ref, s0_ref, s1_ref, m0_ref, m1_ref, qm0_ref, qm1_ref,
               sem_in, sem_x, sem_out):
        cp_wm0 = pltpu.make_async_copy(wmod_hbm.at[:, 0:2 * _D], wmod_ref.at[:, 0:2 * _D], sem_in.at[0])
        cp_x = [pltpu.make_async_copy(x_hbm.at[t * tm:(t + 1) * tm, :], x_ref.at[t * tm:(t + 1) * tm, :], sem_x.at[t])
                for t in range(nx)]
        cp_wqkv = pltpu.make_async_copy(wqkv_hbm, wqkv_ref, sem_in.at[1])
        cp_wm1 = pltpu.make_async_copy(wmod_hbm.at[:, 2 * _D:6 * _D], wmod_ref.at[:, 2 * _D:6 * _D], sem_in.at[2])
        cp_wo = pltpu.make_async_copy(wo_hbm, wo_ref, sem_in.at[3])
        cp_w1 = pltpu.make_async_copy(w1_hbm, w1_ref, sem_in.at[4])
        cp_w2 = pltpu.make_async_copy(w2_hbm, w2_ref, sem_in.at[5])
        cp_wm0.start()
        cp_wqkv.start()
        for cp in cp_x:
            cp.start()
        cp_wm1.start()
        cp_wo.start()
        cp_w1.start()
        cp_w2.start()

        c = c_ref[...].astype(jnp.float32)
        sc = (c * jax.nn.sigmoid(c)).astype(jnp.bfloat16)
        sc16 = jnp.broadcast_to(sc, (16, _D))
        cp_wm0.wait()
        mod_a = jnp.dot(sc16, wmod_ref[:, 0:2 * _D], preferred_element_type=jnp.float32)[0:1]
        sa = mod_a[:, 0:_D]
        ca1 = 1.0 + mod_a[:, _D:2 * _D]
        cp_wqkv.wait()
        wqT = wqkv_ref[:, 0:_D].astype(jnp.float32).T.astype(jnp.bfloat16)
        wvT = wqkv_ref[:, 2 * _D:3 * _D].astype(jnp.float32).T.astype(jnp.bfloat16)
        wk = wqkv_ref[:, _D:2 * _D]
        for t in range(nx):
            cp_x[t].wait()
            rows = slice(t * tm, (t + 1) * tm)
            x = x_ref[rows, :].astype(jnp.float32)
            h = _ln_mod(x, ca1, sa).astype(jnp.bfloat16)
            qT = lax.dot_general(wqT, h, _NT, preferred_element_type=jnp.float32)
            _st_blocks(qT_ref, t * (tm // 128), (qT * (0.25 * _LOG2E)).astype(jnp.bfloat16))
            k = jnp.dot(h, wk, preferred_element_type=jnp.float32).astype(jnp.bfloat16)
            for g in range(4):
                k_ref[g, t * tm // 2:(t + 1) * tm // 2, :] = _pk(k[:, g * 128:(g + 1) * 128])
            vT = lax.dot_general(wvT, h, _NT, preferred_element_type=jnp.float32)
            _st_blocks(vT_ref, t * (tm // 128), vT.astype(jnp.bfloat16))

        nc = S // ck
        nb = tq // 128
        cpb = ck // 128
        row_head = lax.broadcasted_iota(jnp.int32, (64, 128), 0) // (_DH // 2)
        sb = (s0_ref, s1_ref)
        mb = (m0_ref, m1_ref)
        qb = (qm0_ref, qm1_ref)

        def make_qm(t, par):
            h = t % _H
            b0 = (t // _H) * nb
            g0 = pl.multiple_of((h // 8) * 64, 64)
            for i in range(nb):
                qg = qT_ref[b0 + i, pl.ds(g0, 64), :]
                qb[par][i] = jnp.where(row_head == h % 8, qg, jnp.zeros_like(qg))

        def stage_a(t, par, c, mx):
            sl = slice(c * ca, (c + 1) * ca)
            qm = _upk(jnp.concatenate([qb[par][i] for i in range(nb)], axis=1))
            kk = _upk(k_ref[(t % _H) // 8, c * ca // 2:(c + 1) * ca // 2, :])
            s = jnp.dot(kk, qm, preferred_element_type=jnp.float32)
            sb[par][sl, :] = s
            cm = _red8(jnp.max, s)
            return cm if mx is None else jnp.maximum(mx, cm)

        def item(b, par):
            t1 = jnp.minimum(b + 1, T - 1)
            t2 = jnp.minimum(b + 2, T - 1)
            h0 = pl.multiple_of((b % _H) * (_DH // 2), _DH // 2)
            m = jnp.max(mb[par][...], axis=0, keepdims=True)
            mx1 = mb[1 - par][...] if DL > 0 else None
            mx2 = None
            l = None
            acc = None
            na = S // ca
            a_done = 0
            for c in range(nc):
                while a_done < na and a_done * ca <= c * ck:
                    a = a_done
                    if a < na - DL:
                        mx1 = stage_a(t1, 1 - par, DL + a, mx1)
                        if a == na - DL - 1:
                            mb[1 - par][...] = mx1
                    else:
                        mx2 = stage_a(t2, par, a - (na - DL), mx2)
                    a_done += 1
                sl = slice(c * ck, (c + 1) * ck)
                vt = _upk(jnp.concatenate([vT_ref[c * cpb + i, pl.ds(h0, _DH // 2), :] for i in range(cpb)], axis=1))
                nsp = nb if "n" in var else 1
                wn = tq // nsp
                ls, os_ = [], []
                for n in range(nsp):
                    ln = slice(n * wn, (n + 1) * wn)
                    p = jnp.exp2(sb[par][sl, ln] - m[:, ln])
                    pb = p.astype(jnp.bfloat16)
                    ls.append(_red8(jnp.sum, pb.astype(jnp.float32) if "u" in var else p))
                    os_.append(jnp.dot(vt, pb, preferred_element_type=jnp.float32))
                cl = ls[0] if nsp == 1 else jnp.concatenate(ls, axis=1)
                o = os_[0] if nsp == 1 else jnp.concatenate(os_, axis=1)
                l = cl if l is None else l + cl
                acc = o if acc is None else acc + o
            if DL > 0:
                mb[par][...] = mx2
            l = jnp.sum(l, axis=0, keepdims=True)
            o = (acc * (1.0 / l)).astype(jnp.bfloat16)
            b0 = (b // _H) * nb
            for i in range(nb):
                oT_ref[b0 + i, pl.ds(h0, _DH // 2), :] = _pk(o[:, i * 128:(i + 1) * 128])

        make_qm(0, 0)
        make_qm(1, 1)
        mx = None
        for c in range(S // ca):
            mx = stage_a(0, 0, c, mx)
        m0_ref[...] = mx
        mx = None
        for c in range(DL):
            mx = stage_a(1, 1, c, mx)
        if DL > 0:
            m1_ref[...] = mx

        def att_body(it, carry):
            for u in range(U):
                b = it * U + u
                make_qm(jnp.minimum(b + 2, T - 1), u % 2)
                item(b, u % 2)
            return carry

        lax.fori_loop(0, T // U, att_body, 0)

        cp_wm1.wait()
        mod_b = jnp.dot(sc16, wmod_ref[:, 2 * _D:6 * _D], preferred_element_type=jnp.float32)[0:1]
        ga = mod_b[:, 0:_D]
        sb = mod_b[:, _D:2 * _D]
        cb1 = 1.0 + mod_b[:, 2 * _D:3 * _D]
        gb = mod_b[:, 3 * _D:4 * _D]
        cp_wo.wait()
        cp_w1.wait()
        cp_w2.wait()
        b1 = b1_ref[...].astype(jnp.float32)
        b2 = b2_ref[...].astype(jnp.float32)
        cp_out = []
        for t in range(nd):
            rows = slice(t * td, (t + 1) * td)
            oT = jnp.concatenate([oT_ref[t * (td // 128) + i] for i in range(td // 128)], axis=1)
            attn = lax.dot_general(_upk(oT), wo_ref[...], _TN, preferred_element_type=jnp.float32)
            x1 = x_ref[rows, :].astype(jnp.float32) + ga * attn
            h2 = _ln_mod(x1, cb1, sb).astype(jnp.bfloat16)
            u = jnp.dot(h2, w1_ref[...], preferred_element_type=jnp.float32) + b1
            r = jnp.maximum(u, 0.0)
            r = (r * r).astype(jnp.bfloat16)
            f = jnp.dot(r, w2_ref[...], preferred_element_type=jnp.float32) + b2
            out_ref[rows, :] = (x1 + gb * f).astype(out_ref.dtype)
            cp = pltpu.make_async_copy(out_ref.at[rows, :], out_hbm.at[rows, :], sem_out.at[t])
            cp.start()
            cp_out.append(cp)
        for cp in cp_out:
            cp.wait()

    return kernel


def run(A_x, A_wqkv, A_wo, B_x, B_w1, B_b1, B_w2, B_b2, c, w_mod, *, tq=512, ck=128, U=2, td=512, tm=512,
        DL=2, ca=None, var='', flags=None):
    ca = ca or ck
    B, S, D = A_x.shape
    F = B_w1.shape[1]
    hbm = pl.BlockSpec(memory_space=pl.ANY)
    vmem = pl.BlockSpec(memory_space=pltpu.VMEM)
    bf = jnp.bfloat16
    u32 = jnp.uint32
    out = pl.pallas_call(
        make_kernel(S, F, tq, ck, ca, U, td, tm, DL, var),
        in_specs=[hbm, hbm, hbm, hbm, vmem, hbm, vmem, vmem, hbm],
        out_specs=hbm,
        out_shape=jax.ShapeDtypeStruct((S, D), A_x.dtype),
        scratch_shapes=[
            pltpu.VMEM((S, D), bf), pltpu.VMEM((D, 3 * D), bf), pltpu.VMEM((D, D), bf),
            pltpu.VMEM((D, F), bf), pltpu.VMEM((F, D), bf), pltpu.VMEM((D, 6 * D), bf),
            pltpu.VMEM((S, D), bf),
            pltpu.VMEM((S // 128, D // 2, 128), u32), pltpu.VMEM((4, S // 2, 128), u32),
            pltpu.VMEM((S // 128, D // 2, 128), u32), pltpu.VMEM((S // 128, D // 2, 128), u32),
            pltpu.VMEM((S, tq), jnp.float32), pltpu.VMEM((S, tq), jnp.float32),
            pltpu.VMEM((8, tq), jnp.float32), pltpu.VMEM((8, tq), jnp.float32),
            pltpu.VMEM((tq // 128, 64, 128), u32), pltpu.VMEM((tq // 128, 64, 128), u32),
            pltpu.SemaphoreType.DMA((6,)), pltpu.SemaphoreType.DMA((S // tm,)), pltpu.SemaphoreType.DMA((S // td,)),
        ],
        compiler_params=pltpu.CompilerParams(vmem_limit_bytes=100 * 1024 * 1024, flags=flags),
    )(A_x.reshape(S, D), A_wqkv, A_wo, B_w1, B_b1.reshape(1, F), B_w2, B_b2.reshape(1, D), c, w_mod)
    return out.reshape(B, S, D)


@jax.jit
def pallas_adaLN_cond__mha_block__dense_activation_squared_relu__prompt_kernel(
    A_x: jax.Array,
    A_wqkv: jax.Array,
    A_wo: jax.Array,
    B_x: jax.Array,
    B_w1: jax.Array,
    B_b1: jax.Array,
    B_w2: jax.Array,
    B_b2: jax.Array,
    c: jax.Array,
    w_mod: jax.Array,
):
    return run(A_x, A_wqkv, A_wo, B_x, B_w1, B_b1, B_w2, B_b2, c, w_mod, tq=256, DL=4, U=8)
```

```python
import jax
import jax.numpy as jnp
from jax import lax
import jax.experimental.pallas as pl
import jax.experimental.pallas.tpu as pltpu

_D = 512
_H = 32
_DH = 16
_LOG2E = 1.4426950408889634
_EPS = 1e-5
_NT = (((1,), (1,)), ((), ()))
_TN = (((0,), (0,)), ((), ()))


def _ln_mod(x, scale, shift):
    m = jnp.mean(x, axis=-1, keepdims=True)
    xc = x - m
    v = jnp.mean(xc * xc, axis=-1, keepdims=True)
    return xc * lax.rsqrt(v + _EPS) * scale + shift


def _red8(fn, s):
    return fn(s.reshape(s.shape[0] // 8, 8, s.shape[1]), axis=0)


def _pk(v):
    return pltpu.bitcast(v, jnp.uint32)


def _upk(v):
    return pltpu.bitcast(v, jnp.bfloat16)


def _st_blocks(ref, b0, val):
    for i in range(val.shape[1] // 128):
        ref[b0 + i] = _pk(val[:, i * 128:(i + 1) * 128])


def make_kernel(S, F, tq, ck, ca, U, td, tm, DL, late, peel, ph, pipeP, pipeD):
    nx = S // tm
    nd = S // td
    T = (S // tq) * _H

    def kernel(x_hbm, wqkv_hbm, wo_hbm, w1_hbm, b1_ref, w2_hbm, b2_ref, c_ref, wmod_hbm,
               out_hbm,
               x_ref, wqkv_ref, wo_ref, w1_ref, w2_ref, wmod_ref, out_ref,
               qT_ref, k_ref, vT_ref, oT_ref, s0_ref, s1_ref, m0_ref, m1_ref, qm0_ref, qm1_ref,
               sem_in, sem_x, sem_out):
        cp_wm0 = pltpu.make_async_copy(wmod_hbm.at[:, 0:2 * _D], wmod_ref.at[:, 0:2 * _D], sem_in.at[0])
        cp_x = [pltpu.make_async_copy(x_hbm.at[t * tm:(t + 1) * tm, :], x_ref.at[t * tm:(t + 1) * tm, :], sem_x.at[t])
                for t in range(nx)]
        cp_w = [pltpu.make_async_copy(wqkv_hbm.at[:, j * _D:(j + 1) * _D], wqkv_ref.at[:, j * _D:(j + 1) * _D],
                                      sem_in.at[6 + j]) for j in range(3)]
        cp_wm1 = pltpu.make_async_copy(wmod_hbm.at[:, 2 * _D:6 * _D], wmod_ref.at[:, 2 * _D:6 * _D], sem_in.at[2])
        cp_wo = pltpu.make_async_copy(wo_hbm, wo_ref, sem_in.at[3])
        cp_w1 = pltpu.make_async_copy(w1_hbm, w1_ref, sem_in.at[4])
        cp_w2 = pltpu.make_async_copy(w2_hbm, w2_ref, sem_in.at[5])
        cp_wm0.start()
        cp_x[0].start()
        cp_w[1].start()
        if late == 0:
            cp_w[0].start()
            cp_w[2].start()
            for cp in cp_x[1:]:
                cp.start()

        c = c_ref[...].astype(jnp.float32)
        sc = (c * jax.nn.sigmoid(c)).astype(jnp.bfloat16)
        sc16 = jnp.broadcast_to(sc, (16, _D))
        cp_wm0.wait()
        if late > 0:
            cp_w[0].start()
            cp_w[2].start()
        if late == 1:
            for cp in cp_x[1:]:
                cp.start()
        mod_a = jnp.dot(sc16, wmod_ref[:, 0:2 * _D], preferred_element_type=jnp.float32)[0:1]
        sa = mod_a[:, 0:_D]
        ca1 = 1.0 + mod_a[:, _D:2 * _D]
        def ln_a(t):
            cp_x[t].wait()
            x = x_ref[t * tm:(t + 1) * tm, :].astype(jnp.float32)
            return _ln_mod(x, ca1, sa).astype(jnp.bfloat16)

        h_next = ln_a(0)
        for t in range(nx):
            h = h_next
            if pipeP and t == 0:
                cp_w[1].wait()
                if late == 2:
                    for cp in cp_x[1:]:
                        cp.start()
            if pipeP and t + 1 < nx and (t > 0 or pipeP > 1):
                h_next = ln_a(t + 1)
            if t == 0 and not pipeP:
                cp_w[1].wait()
                if late == 2:
                    for cp in cp_x[1:]:
                        cp.start()
            k = jnp.dot(h, wqkv_ref[:, _D:2 * _D], preferred_element_type=jnp.float32).astype(jnp.bfloat16)
            for g in range(4):
                k_ref[g, t * tm // 2:(t + 1) * tm // 2, :] = _pk(k[:, g * 128:(g + 1) * 128])
            if t == 0:
                cp_w[0].wait()
                if 'q' not in ph:
                    wqT = wqkv_ref[:, 0:_D].astype(jnp.float32).T.astype(jnp.bfloat16)
            if 'q' in ph:
                qT = jnp.dot(h, wqkv_ref[:, 0:_D], preferred_element_type=jnp.float32).T
            else:
                qT = lax.dot_general(wqT, h, _NT, preferred_element_type=jnp.float32)
            _st_blocks(qT_ref, t * (tm // 128), (qT * (0.25 * _LOG2E)).astype(jnp.bfloat16))
            if t == 0:
                cp_w[2].wait()
                cp_wo.start()
                cp_wm1.start()
                cp_w1.start()
                cp_w2.start()
                if 'v' not in ph:
                    wvT = wqkv_ref[:, 2 * _D:3 * _D].astype(jnp.float32).T.astype(jnp.bfloat16)
            if 'v' in ph:
                vT = jnp.dot(h, wqkv_ref[:, 2 * _D:3 * _D], preferred_element_type=jnp.float32).T
            else:
                vT = lax.dot_general(wvT, h, _NT, preferred_element_type=jnp.float32)
            _st_blocks(vT_ref, t * (tm // 128), vT.astype(jnp.bfloat16))
            if t + 1 < nx and (not pipeP or (t == 0 and pipeP == 1)):
                h_next = ln_a(t + 1)

        nc = S // ck
        nb = tq // 128
        cpb = ck // 128
        row_head = lax.broadcasted_iota(jnp.int32, (64, 128), 0) // (_DH // 2)
        sb = (s0_ref, s1_ref)
        mb = (m0_ref, m1_ref)
        qb = (qm0_ref, qm1_ref)

        def make_qm(t, par):
            h = t % _H
            b0 = (t // _H) * nb
            g0 = pl.multiple_of((h // 8) * 64, 64)
            for i in range(nb):
                qg = qT_ref[b0 + i, pl.ds(g0, 64), :]
                qb[par][i] = jnp.where(row_head == h % 8, qg, jnp.zeros_like(qg))

        def stage_a(t, par, c, mx):
            sl = slice(c * ca, (c + 1) * ca)
            qm = _upk(jnp.concatenate([qb[par][i] for i in range(nb)], axis=1))
            kk = _upk(k_ref[(t % _H) // 8, c * ca // 2:(c + 1) * ca // 2, :])
            s = jnp.dot(kk, qm, preferred_element_type=jnp.float32)
            sb[par][sl, :] = s
            cm = _red8(jnp.max, s)
            return cm if mx is None else jnp.maximum(mx, cm)

        def item(b, par, has1=True, has2=True):
            t1 = b + 1 if peel else jnp.minimum(b + 1, T - 1)
            t2 = b + 2 if peel else jnp.minimum(b + 2, T - 1)
            h0 = pl.multiple_of((b % _H) * (_DH // 2), _DH // 2)
            m = jnp.max(mb[par][...], axis=0, keepdims=True)
            mx1 = mb[1 - par][...] if (DL > 0 and has1) else None
            mx2 = None
            l = None
            acc = None
            na = S // ca
            a_done = 0
            for c in range(nc):
                while a_done < na and a_done * ca <= c * ck:
                    a = a_done
                    if a < na - DL:
                        if has1:
                            mx1 = stage_a(t1, 1 - par, DL + a, mx1)
                            if a == na - DL - 1:
                                mb[1 - par][...] = mx1
                    elif has2:
                        mx2 = stage_a(t2, par, a - (na - DL), mx2)
                    a_done += 1
                sl = slice(c * ck, (c + 1) * ck)
                p = jnp.exp2(sb[par][sl, :] - m)
                cl = _red8(jnp.sum, p)
                l = cl if l is None else l + cl
                vt = _upk(jnp.concatenate([vT_ref[c * cpb + i, pl.ds(h0, _DH // 2), :] for i in range(cpb)], axis=1))
                o = jnp.dot(vt, p.astype(jnp.bfloat16), preferred_element_type=jnp.float32)
                acc = o if acc is None else acc + o
            if DL > 0 and has2:
                mb[par][...] = mx2
            l = jnp.sum(l, axis=0, keepdims=True)
            o = (acc * (1.0 / l)).astype(jnp.bfloat16)
            b0 = (b // _H) * nb
            for i in range(nb):
                oT_ref[b0 + i, pl.ds(h0, _DH // 2), :] = _pk(o[:, i * 128:(i + 1) * 128])

        make_qm(0, 0)
        make_qm(1, 1)
        mx = None
        for c in range(S // ca):
            mx = stage_a(0, 0, c, mx)
        m0_ref[...] = mx
        mx = None
        for c in range(DL):
            mx = stage_a(1, 1, c, mx)
        if DL > 0:
            m1_ref[...] = mx

        def att_body(it, carry):
            for u in range(U):
                b = it * U + u
                make_qm(b + 2 if peel else jnp.minimum(b + 2, T - 1), u % 2)
                item(b, u % 2)
            return carry

        if 'A' not in ph:
            cp_wm1.wait(); cp_wo.wait(); cp_w1.wait(); cp_w2.wait()
            cp = pltpu.make_async_copy(out_ref.at[0:16, :], out_hbm.at[0:16, :], sem_out.at[0])
            cp.start(); cp.wait()
            return
        n_main = (T - 2) // U if peel else T // U
        lax.fori_loop(0, n_main, att_body, 0)
        for b in range(n_main * U, T):
            if b + 2 < T:
                make_qm(b + 2, b % 2)
            item(b, b % 2, b + 1 < T, b + 2 < T)

        cp_wm1.wait()
        mod_b = jnp.dot(sc16, wmod_ref[:, 2 * _D:6 * _D], preferred_element_type=jnp.float32)[0:1]
        ga = mod_b[:, 0:_D]
        sb = mod_b[:, _D:2 * _D]
        cb1 = 1.0 + mod_b[:, 2 * _D:3 * _D]
        gb = mod_b[:, 3 * _D:4 * _D]
        cp_wo.wait()
        cp_w1.wait()
        cp_w2.wait()
        b1 = b1_ref[...].astype(jnp.float32).reshape(1, F)
        b2 = b2_ref[...].astype(jnp.float32).reshape(1, _D)
        cp_out = []
        def d1(t):
            rows = slice(t * td, (t + 1) * td)
            oT = jnp.concatenate([oT_ref[t * (td // 128) + i] for i in range(td // 128)], axis=1)
            attn = lax.dot_general(_upk(oT), wo_ref[...], _TN, preferred_element_type=jnp.float32)
            x1 = x_ref[rows, :].astype(jnp.float32) + ga * attn
            return x1, _ln_mod(x1, cb1, sb).astype(jnp.bfloat16)

        nxt = d1(0)
        for t in range(nd):
            rows = slice(t * td, (t + 1) * td)
            x1, h2 = nxt
            if pipeD and t + 1 < nd:
                nxt = d1(t + 1)
            u = jnp.dot(h2, w1_ref[...], preferred_element_type=jnp.float32) + b1
            r = jnp.maximum(u, 0.0)
            r = (r * r).astype(jnp.bfloat16)
            f = jnp.dot(r, w2_ref[...], preferred_element_type=jnp.float32) + b2
            out_ref[rows, :] = (x1 + gb * f).astype(out_ref.dtype)
            cp = pltpu.make_async_copy(out_ref.at[rows, :], out_hbm.at[rows, :], sem_out.at[t])
            cp.start()
            cp_out.append(cp)
            if not pipeD and t + 1 < nd:
                nxt = d1(t + 1)
        for cp in cp_out:
            cp.wait()

    return kernel


def run(A_x, A_wqkv, A_wo, B_x, B_w1, B_b1, B_w2, B_b2, c, w_mod, *, tq=256, ck=128, U=16, td=512, tm=512,
        DL=4, ca=None, late=2, peel=False, ph='PADqv', pipeP=1, pipeD=True, b1d=True, flags=None):
    ca = ca or ck
    B, S, D = A_x.shape
    F = B_w1.shape[1]
    hbm = pl.BlockSpec(memory_space=pl.ANY)
    vmem = pl.BlockSpec(memory_space=pltpu.VMEM)
    bf = jnp.bfloat16
    u32 = jnp.uint32
    out = pl.pallas_call(
        make_kernel(S, F, tq, ck, ca, U, td, tm, DL, late, peel, ph, pipeP, pipeD),
        in_specs=[hbm, hbm, hbm, hbm, vmem, hbm, vmem, vmem, hbm],
        out_specs=hbm,
        out_shape=jax.ShapeDtypeStruct((S, D), A_x.dtype),
        scratch_shapes=[
            pltpu.VMEM((S, D), bf), pltpu.VMEM((D, 3 * D), bf), pltpu.VMEM((D, D), bf),
            pltpu.VMEM((D, F), bf), pltpu.VMEM((F, D), bf), pltpu.VMEM((D, 6 * D), bf),
            pltpu.VMEM((S, D), bf),
            pltpu.VMEM((S // 128, D // 2, 128), u32), pltpu.VMEM((4, S // 2, 128), u32),
            pltpu.VMEM((S // 128, D // 2, 128), u32), pltpu.VMEM((S // 128, D // 2, 128), u32),
            pltpu.VMEM((S, tq), jnp.float32), pltpu.VMEM((S, tq), jnp.float32),
            pltpu.VMEM((8, tq), jnp.float32), pltpu.VMEM((8, tq), jnp.float32),
            pltpu.VMEM((tq // 128, 64, 128), u32), pltpu.VMEM((tq // 128, 64, 128), u32),
            pltpu.SemaphoreType.DMA((9,)), pltpu.SemaphoreType.DMA((S // tm,)), pltpu.SemaphoreType.DMA((S // td,)),
        ],
        compiler_params=pltpu.CompilerParams(vmem_limit_bytes=100 * 1024 * 1024, flags=flags),
    )(A_x.reshape(S, D), A_wqkv, A_wo, B_w1, B_b1 if b1d else B_b1.reshape(1, F), B_w2, B_b2 if b1d else B_b2.reshape(1, D), c, w_mod)
    return out.reshape(B, S, D)


@jax.jit
def pallas_adaLN_cond__mha_block__dense_activation_squared_relu__prompt_kernel(
    A_x: jax.Array,
    A_wqkv: jax.Array,
    A_wo: jax.Array,
    B_x: jax.Array,
    B_w1: jax.Array,
    B_b1: jax.Array,
    B_w2: jax.Array,
    B_b2: jax.Array,
    c: jax.Array,
    w_mod: jax.Array,
):
    return run(A_x, A_wqkv, A_wo, B_x, B_w1, B_b1, B_w2, B_b2, c, w_mod, U=28, peel=True)
```

```python
import jax
import jax.numpy as jnp
from jax import lax
import jax.experimental.pallas as pl
import jax.experimental.pallas.tpu as pltpu

_D = 512
_H = 32
_DH = 16
_EPS = 1e-5
_QSCALE = 0.25 * 1.4426950408889634
_TN = (((0,), (0,)), ((), ()))


def _ln_mod(x, scale, shift):
    m = jnp.mean(x, axis=-1, keepdims=True)
    xc = x - m
    v = jnp.mean(xc * xc, axis=-1, keepdims=True)
    return xc * lax.rsqrt(v + _EPS) * scale + shift


def _red8(fn, s):
    return fn(s.reshape(s.shape[0] // 8, 8, s.shape[1]), axis=0)


def _pk(v):
    return pltpu.bitcast(v, jnp.uint32)


def _upk(v):
    return pltpu.bitcast(v, jnp.bfloat16)


def _offs(sizes):
    o = [0]
    for z in sizes:
        o.append(o[-1] + z)
    return [(o[i], o[i + 1]) for i in range(len(sizes))]


def _make_kernel(S, F, tq, ck, U, lag, pt, dt, early, small_dma):
    nx, nd = len(pt), len(dt)
    T = (S // tq) * _H
    nc, nb = S // ck, tq // 128

    def kernel(x_hbm, wqkv_hbm, wo_hbm, w1_hbm, b1_in, w2_hbm, b2_in, c_in, wmod_hbm, out_hbm,
               x_ref, wq_ref, wk_ref, wv_ref, wo_ref, w1_ref, w2_ref, wma_ref, wmb_ref, out_ref,
               qT_ref, k_ref, vT_ref, oT_ref, s0_ref, s1_ref, m0_ref, m1_ref, qm0_ref, qm1_ref,
               b1_scr, b2_scr, c_scr, sem_in, sem_x, sem_out):
        def cp_in(i, src, dst):
            return pltpu.make_async_copy(src, dst, sem_in.at[i])

        cp_wma = cp_in(0, wmod_hbm.at[:, 0:2 * _D], wma_ref)
        cp_wmb = cp_in(1, wmod_hbm.at[:, 2 * _D:6 * _D], wmb_ref)
        cp_wq, cp_wk, cp_wv = [cp_in(2 + j, wqkv_hbm.at[:, j * _D:(j + 1) * _D], r)
                               for j, r in enumerate((wq_ref, wk_ref, wv_ref))]
        cp_wo, cp_w1, cp_w2 = cp_in(5, wo_hbm, wo_ref), cp_in(6, w1_hbm, w1_ref), cp_in(7, w2_hbm, w2_ref)
        cp_x = [pltpu.make_async_copy(x_hbm.at[r0:r1, :], x_ref.at[r0:r1, :], sem_x.at[t])
                for t, (r0, r1) in enumerate(pt)]
        if small_dma:
            cp_c, cp_b1, cp_b2 = cp_in(8, c_in, c_scr), cp_in(9, b1_in, b1_scr), cp_in(10, b2_in, b2_scr)
            cp_c.start()
            c_ref, b1_ref, b2_ref = c_scr, b1_scr, b2_scr
        else:
            c_ref, b1_ref, b2_ref = c_in, b1_in, b2_in
        cp_wma.start()
        cp_x[0].start()
        cp_wk.start()

        if small_dma:
            cp_c.wait()
        c = c_ref[...].astype(jnp.float32)
        sc16 = jnp.broadcast_to((c * jax.nn.sigmoid(c)).astype(jnp.bfloat16), (16, _D))
        cp_wma.wait()
        cp_wq.start()
        cp_wv.start()
        mod_a = jnp.dot(sc16, wma_ref[...], preferred_element_type=jnp.float32)[0:1]
        sa = mod_a[:, 0:_D]
        ca1 = 1.0 + mod_a[:, _D:2 * _D]

        def ln_a(t):
            cp_x[t].wait()
            x = x_ref[pt[t][0]:pt[t][1], :].astype(jnp.float32)
            return _ln_mod(x, ca1, sa).astype(jnp.bfloat16)

        def st_blocks(ref, b0, val):
            for i in range(val.shape[1] // 128):
                ref[b0 + i] = _pk(val[:, i * 128:(i + 1) * 128])

        h_next = ln_a(0)
        cp_wk.wait()
        for cp in cp_x[1:]:
            cp.start()
        for t, (r0, r1) in enumerate(pt):
            h = h_next
            if 0 < t < nx - 1:
                h_next = ln_a(t + 1)
            k = jnp.dot(h, wk_ref[...], preferred_element_type=jnp.float32).astype(jnp.bfloat16)
            for g in range(4):
                k_ref[g, r0 // 2:r1 // 2, :] = _pk(k[:, g * 128:(g + 1) * 128])
            if t == 0:
                cp_wq.wait()
            qT = jnp.dot(h, wq_ref[...], preferred_element_type=jnp.float32).T
            st_blocks(qT_ref, r0 // 128, (qT * _QSCALE).astype(jnp.bfloat16))
            if t == 0:
                cp_wv.wait()
                for cp in (cp_wo, cp_wmb, cp_w1, cp_w2) + ((cp_b1, cp_b2) if small_dma else ()):
                    cp.start()
            vT = jnp.dot(h, wv_ref[...], preferred_element_type=jnp.float32).T
            st_blocks(vT_ref, r0 // 128, vT.astype(jnp.bfloat16))
            if t == 0 and nx > 1:
                h_next = ln_a(1)

        row_head = lax.broadcasted_iota(jnp.int32, (64, 128), 0) // (_DH // 2)
        sbuf, mbuf, qbuf = (s0_ref, s1_ref), (m0_ref, m1_ref), (qm0_ref, qm1_ref)

        def make_qm(t, par):
            h = t % _H
            g0 = pl.multiple_of((h // 8) * 64, 64)
            for i in range(nb):
                qg = qT_ref[(t // _H) * nb + i, pl.ds(g0, 64), :]
                qbuf[par][i] = jnp.where(row_head == h % 8, qg, jnp.zeros_like(qg))

        def stage_a(t, par, c, mx):
            qm = _upk(jnp.concatenate([qbuf[par][i] for i in range(nb)], axis=1))
            kk = _upk(k_ref[(t % _H) // 8, c * ck // 2:(c + 1) * ck // 2, :])
            s = jnp.dot(kk, qm, preferred_element_type=jnp.float32)
            sbuf[par][c * ck:(c + 1) * ck, :] = s
            cm = _red8(jnp.max, s)
            return cm if mx is None else jnp.maximum(mx, cm)

        def item(b, par, has1=True, has2=True):
            h0 = pl.multiple_of((b % _H) * (_DH // 2), _DH // 2)
            m = jnp.max(mbuf[par][...], axis=0, keepdims=True)
            mx1 = mbuf[1 - par][...] if has1 else None
            mx2 = l = acc = None
            for c in range(nc):
                if c < nc - lag:
                    if has1:
                        mx1 = stage_a(b + 1, 1 - par, lag + c, mx1)
                        if c == nc - lag - 1:
                            mbuf[1 - par][...] = mx1
                elif has2:
                    mx2 = stage_a(b + 2, par, c - (nc - lag), mx2)
                p = jnp.exp2(sbuf[par][c * ck:(c + 1) * ck, :] - m)
                cl = _red8(jnp.sum, p)
                l = cl if l is None else l + cl
                vt = _upk(jnp.concatenate(
                    [vT_ref[c * (ck // 128) + i, pl.ds(h0, _DH // 2), :] for i in range(ck // 128)], axis=1))
                o = jnp.dot(vt, p.astype(jnp.bfloat16), preferred_element_type=jnp.float32)
                acc = o if acc is None else acc + o
            if has2:
                mbuf[par][...] = mx2
            o = (acc * (1.0 / jnp.sum(l, axis=0, keepdims=True))).astype(jnp.bfloat16)
            for i in range(nb):
                oT_ref[(b // _H) * nb + i, pl.ds(h0, _DH // 2), :] = _pk(o[:, i * 128:(i + 1) * 128])

        make_qm(0, 0)
        make_qm(1, 1)
        mx = None
        for c in range(nc):
            mx = stage_a(0, 0, c, mx)
        m0_ref[...] = mx
        mx = None
        for c in range(lag):
            mx = stage_a(1, 1, c, mx)
        m1_ref[...] = mx

        def att_body(it, carry):
            for u in range(U):
                b = it * U + u
                make_qm(b + 2, u % 2)
                item(b, u % 2)
            return carry

        n_main = (T - 2) // U
        lax.fori_loop(0, n_main, att_body, 0)

        for cp in (cp_wmb, cp_wo, cp_w1, cp_w2) + ((cp_b1, cp_b2) if small_dma else ()):
            cp.wait()
        mod_b = jnp.dot(sc16, wmb_ref[...], preferred_element_type=jnp.float32)[0:1]
        ga, shb = mod_b[:, 0:_D], mod_b[:, _D:2 * _D]
        cb1, gb = 1.0 + mod_b[:, 2 * _D:3 * _D], mod_b[:, 3 * _D:4 * _D]
        b1 = b1_ref[...].astype(jnp.float32).reshape(1, F)
        b2 = b2_ref[...].astype(jnp.float32).reshape(1, _D)

        def d1(t):
            r0, r1 = dt[t]
            oT = jnp.concatenate([oT_ref[i] for i in range(r0 // 128, r1 // 128)], axis=1)
            attn = lax.dot_general(_upk(oT), wo_ref[...], _TN, preferred_element_type=jnp.float32)
            x1 = x_ref[r0:r1, :].astype(jnp.float32) + ga * attn
            return x1, _ln_mod(x1, cb1, shb).astype(jnp.bfloat16)

        nxt = None
        for b in range(n_main * U, T):
            if b + 2 < T:
                make_qm(b + 2, b % 2)
            if b == T - early:
                nxt = d1(0)
            item(b, b % 2, b + 1 < T, b + 2 < T)
        if nxt is None:
            nxt = d1(0)

        cp_out = []
        for t, (r0, r1) in enumerate(dt):
            x1, h2 = nxt
            if t + 1 < nd:
                nxt = d1(t + 1)
            u = jnp.dot(h2, w1_ref[...], preferred_element_type=jnp.float32) + b1
            r = jnp.maximum(u, 0.0)
            f = jnp.dot((r * r).astype(jnp.bfloat16), w2_ref[...], preferred_element_type=jnp.float32) + b2
            out_ref[r0:r1, :] = (x1 + gb * f).astype(out_ref.dtype)
            cp = pltpu.make_async_copy(out_ref.at[r0:r1, :], out_hbm.at[r0:r1, :], sem_out.at[t])
            cp.start()
            cp_out.append(cp)
        for cp in cp_out:
            cp.wait()

    return kernel


def run(A_x, A_wqkv, A_wo, B_x, B_w1, B_b1, B_w2, B_b2, c, w_mod, *, tq=256, ck=128, U=28, lag=4,
        tm=(512, 512, 512, 512), td=(512, 512, 512, 256, 256), early=1, small_dma=False):
    del B_x
    B, S, D = A_x.shape
    F = B_w1.shape[1]
    assert (B, D) == (1, _D) and sum(tm) == S and sum(td) == S and U % 2 == 0 and 0 < lag <= S // ck // 2
    hbm = pl.BlockSpec(memory_space=pl.ANY)
    small = hbm if small_dma else pl.BlockSpec(memory_space=pltpu.VMEM)
    bf, u32, f32, V = jnp.bfloat16, jnp.uint32, jnp.float32, pltpu.VMEM
    out = pl.pallas_call(
        _make_kernel(S, F, tq, ck, U, lag, _offs(tm), _offs(td), early, small_dma),
        in_specs=[hbm, hbm, hbm, hbm, small, hbm, small, small, hbm],
        out_specs=hbm,
        out_shape=jax.ShapeDtypeStruct((S, D), A_x.dtype),
        scratch_shapes=[
            V((S, D), bf), V((D, D), bf), V((D, D), bf), V((D, D), bf), V((D, D), bf),
            V((D, F), bf), V((F, D), bf), V((D, 2 * D), bf), V((D, 4 * D), bf), V((S, D), bf),
            V((S // 128, D // 2, 128), u32), V((4, S // 2, 128), u32),
            V((S // 128, D // 2, 128), u32), V((S // 128, D // 2, 128), u32),
            V((S, tq), f32), V((S, tq), f32), V((8, tq), f32), V((8, tq), f32),
            V((tq // 128, 64, 128), u32), V((tq // 128, 64, 128), u32),
            V((F,), bf), V((D,), bf), V((1, D), bf),
            pltpu.SemaphoreType.DMA((11,)), pltpu.SemaphoreType.DMA((len(tm),)),
            pltpu.SemaphoreType.DMA((len(td),)),
        ],
        compiler_params=pltpu.CompilerParams(vmem_limit_bytes=100 * 1024 * 1024),
    )(A_x.reshape(S, D), A_wqkv, A_wo, B_w1, B_b1, B_w2, B_b2, c, w_mod)
    return out.reshape(B, S, D)


@jax.jit
def pallas_adaLN_cond__mha_block__dense_activation_squared_relu__prompt_kernel(
    A_x: jax.Array,
    A_wqkv: jax.Array,
    A_wo: jax.Array,
    B_x: jax.Array,
    B_w1: jax.Array,
    B_b1: jax.Array,
    B_w2: jax.Array,
    B_b2: jax.Array,
    c: jax.Array,
    w_mod: jax.Array,
):
    return run(A_x, A_wqkv, A_wo, B_x, B_w1, B_b1, B_w2, B_b2, c, w_mod, small_dma=True)
```

```python
import jax
import jax.numpy as jnp
from jax import lax
import jax.experimental.pallas as pl
import jax.experimental.pallas.tpu as pltpu

_D = 512
_H = 32
_DH = 16
_EPS = 1e-5
_QSCALE = 0.25 * 1.4426950408889634
_TN = (((0,), (0,)), ((), ()))


def _ln_mod(x, scale, shift):
    m = jnp.mean(x, axis=-1, keepdims=True)
    xc = x - m
    v = jnp.mean(xc * xc, axis=-1, keepdims=True)
    return xc * lax.rsqrt(v + _EPS) * scale + shift


def _red8(fn, s):
    return fn(s.reshape(s.shape[0] // 8, 8, s.shape[1]), axis=0)


def _pk(v):
    return pltpu.bitcast(v, jnp.uint32)


def _upk(v):
    return pltpu.bitcast(v, jnp.bfloat16)


def _offs(sizes):
    o = [0]
    for z in sizes:
        o.append(o[-1] + z)
    return [(o[i], o[i + 1]) for i in range(len(sizes))]


def _make_kernel(S, F, tq, ck, U, lag, pt, dt, early):
    nx, nd = len(pt), len(dt)
    T = (S // tq) * _H
    nc, nb = S // ck, tq // 128

    def kernel(x_hbm, wqkv_hbm, wo_hbm, w1_hbm, b1_hbm, w2_hbm, b2_hbm, c_hbm, wmod_hbm, out_hbm,
               x_ref, wq_ref, wk_ref, wv_ref, wo_ref, w1_ref, w2_ref, wma_ref, wmb_ref, out_ref,
               qT_ref, k_ref, vT_ref, oT_ref, s0_ref, s1_ref, m0_ref, m1_ref, qm0_ref, qm1_ref,
               b1_ref, b2_ref, c_ref, sem_in, sem_x, sem_out):
        def cp_in(i, src, dst):
            return pltpu.make_async_copy(src, dst, sem_in.at[i])

        cp_wma = cp_in(0, wmod_hbm.at[:, 0:2 * _D], wma_ref)
        cp_wmb = cp_in(1, wmod_hbm.at[:, 2 * _D:6 * _D], wmb_ref)
        cp_wq, cp_wk, cp_wv = [cp_in(2 + j, wqkv_hbm.at[:, j * _D:(j + 1) * _D], r)
                               for j, r in enumerate((wq_ref, wk_ref, wv_ref))]
        cp_wo, cp_w1, cp_w2 = cp_in(5, wo_hbm, wo_ref), cp_in(6, w1_hbm, w1_ref), cp_in(7, w2_hbm, w2_ref)
        cp_x = [pltpu.make_async_copy(x_hbm.at[r0:r1, :], x_ref.at[r0:r1, :], sem_x.at[t])
                for t, (r0, r1) in enumerate(pt)]
        cp_c, cp_b1, cp_b2 = cp_in(8, c_hbm, c_ref), cp_in(9, b1_hbm, b1_ref), cp_in(10, b2_hbm, b2_ref)
        cp_c.start()
        cp_wma.start()
        cp_x[0].start()
        cp_wk.start()

        cp_c.wait()
        c = c_ref[...].astype(jnp.float32)
        sc16 = jnp.broadcast_to((c * jax.nn.sigmoid(c)).astype(jnp.bfloat16), (16, _D))
        cp_wma.wait()
        cp_wq.start()
        cp_wv.start()
        mod_a = jnp.dot(sc16, wma_ref[...], preferred_element_type=jnp.float32)[0:1]
        sa = mod_a[:, 0:_D]
        ca1 = 1.0 + mod_a[:, _D:2 * _D]

        def ln_a(t):
            cp_x[t].wait()
            x = x_ref[pt[t][0]:pt[t][1], :].astype(jnp.float32)
            return _ln_mod(x, ca1, sa).astype(jnp.bfloat16)

        def st_blocks(ref, b0, val):
            for i in range(val.shape[1] // 128):
                ref[b0 + i] = _pk(val[:, i * 128:(i + 1) * 128])

        h_next = ln_a(0)
        cp_wk.wait()
        for cp in cp_x[1:]:
            cp.start()
        for t, (r0, r1) in enumerate(pt):
            h = h_next
            if 0 < t < nx - 1:
                h_next = ln_a(t + 1)
            k = jnp.dot(h, wk_ref[...], preferred_element_type=jnp.float32).astype(jnp.bfloat16)
            for g in range(4):
                k_ref[g, r0 // 2:r1 // 2, :] = _pk(k[:, g * 128:(g + 1) * 128])
            if t == 0:
                cp_wq.wait()
            qT = jnp.dot(h, wq_ref[...], preferred_element_type=jnp.float32).T
            st_blocks(qT_ref, r0 // 128, (qT * _QSCALE).astype(jnp.bfloat16))
            if t == 0:
                cp_wv.wait()
                for cp in (cp_wo, cp_wmb, cp_w1, cp_w2, cp_b1, cp_b2):
                    cp.start()
            vT = jnp.dot(h, wv_ref[...], preferred_element_type=jnp.float32).T
            st_blocks(vT_ref, r0 // 128, vT.astype(jnp.bfloat16))
            if t == 0 and nx > 1:
                h_next = ln_a(1)

        row_head = lax.broadcasted_iota(jnp.int32, (64, 128), 0) // (_DH // 2)
        sbuf, mbuf, qbuf = (s0_ref, s1_ref), (m0_ref, m1_ref), (qm0_ref, qm1_ref)

        def make_qm(t, par):
            h = t % _H
            g0 = pl.multiple_of((h // 8) * 64, 64)
            for i in range(nb):
                qg = qT_ref[(t // _H) * nb + i, pl.ds(g0, 64), :]
                qbuf[par][i] = jnp.where(row_head == h % 8, qg, jnp.zeros_like(qg))

        def stage_a(t, par, c, mx):
            qm = _upk(jnp.concatenate([qbuf[par][i] for i in range(nb)], axis=1))
            kk = _upk(k_ref[(t % _H) // 8, c * ck // 2:(c + 1) * ck // 2, :])
            s = jnp.dot(kk, qm, preferred_element_type=jnp.float32)
            sbuf[par][c * ck:(c + 1) * ck, :] = s
            cm = _red8(jnp.max, s)
            return cm if mx is None else jnp.maximum(mx, cm)

        def item(b, par, has1=True, has2=True):
            h0 = pl.multiple_of((b % _H) * (_DH // 2), _DH // 2)
            m = jnp.max(mbuf[par][...], axis=0, keepdims=True)
            mx1 = mbuf[1 - par][...] if has1 else None
            mx2 = l = acc = None
            for c in range(nc):
                if c < nc - lag:
                    if has1:
                        mx1 = stage_a(b + 1, 1 - par, lag + c, mx1)
                        if c == nc - lag - 1:
                            mbuf[1 - par][...] = mx1
                elif has2:
                    mx2 = stage_a(b + 2, par, c - (nc - lag), mx2)
                p = jnp.exp2(sbuf[par][c * ck:(c + 1) * ck, :] - m)
                cl = _red8(jnp.sum, p)
                l = cl if l is None else l + cl
                vt = _upk(jnp.concatenate(
                    [vT_ref[c * (ck // 128) + i, pl.ds(h0, _DH // 2), :] for i in range(ck // 128)], axis=1))
                o = jnp.dot(vt, p.astype(jnp.bfloat16), preferred_element_type=jnp.float32)
                acc = o if acc is None else acc + o
            if has2:
                mbuf[par][...] = mx2
            o = (acc * (1.0 / jnp.sum(l, axis=0, keepdims=True))).astype(jnp.bfloat16)
            for i in range(nb):
                oT_ref[(b // _H) * nb + i, pl.ds(h0, _DH // 2), :] = _pk(o[:, i * 128:(i + 1) * 128])

        make_qm(0, 0)
        make_qm(1, 1)
        mx = None
        for c in range(nc):
            mx = stage_a(0, 0, c, mx)
        m0_ref[...] = mx
        mx = None
        for c in range(lag):
            mx = stage_a(1, 1, c, mx)
        m1_ref[...] = mx

        def att_body(it, carry):
            for u in range(U):
                b = it * U + u
                make_qm(b + 2, u % 2)
                item(b, u % 2)
            return carry

        n_main = (T - 2) // U
        lax.fori_loop(0, n_main, att_body, 0)

        for cp in (cp_wmb, cp_wo, cp_w1, cp_w2, cp_b1, cp_b2):
            cp.wait()
        mod_b = jnp.dot(sc16, wmb_ref[...], preferred_element_type=jnp.float32)[0:1]
        ga, shb = mod_b[:, 0:_D], mod_b[:, _D:2 * _D]
        cb1, gb = 1.0 + mod_b[:, 2 * _D:3 * _D], mod_b[:, 3 * _D:4 * _D]
        b1 = b1_ref[...].astype(jnp.float32).reshape(1, F)
        b2 = b2_ref[...].astype(jnp.float32).reshape(1, _D)

        def d1(t):
            r0, r1 = dt[t]
            oT = jnp.concatenate([oT_ref[i] for i in range(r0 // 128, r1 // 128)], axis=1)
            attn = lax.dot_general(_upk(oT), wo_ref[...], _TN, preferred_element_type=jnp.float32)
            x1 = x_ref[r0:r1, :].astype(jnp.float32) + ga * attn
            return x1, _ln_mod(x1, cb1, shb).astype(jnp.bfloat16)

        nxt = None
        for b in range(n_main * U, T):
            if b + 2 < T:
                make_qm(b + 2, b % 2)
            if b == T - early:
                nxt = d1(0)
            item(b, b % 2, b + 1 < T, b + 2 < T)
        if nxt is None:
            nxt = d1(0)

        cp_out = []
        for t, (r0, r1) in enumerate(dt):
            x1, h2 = nxt
            if t + 1 < nd:
                nxt = d1(t + 1)
            u = jnp.dot(h2, w1_ref[...], preferred_element_type=jnp.float32) + b1
            r = jnp.maximum(u, 0.0)
            f = jnp.dot((r * r).astype(jnp.bfloat16), w2_ref[...], preferred_element_type=jnp.float32) + b2
            out_ref[r0:r1, :] = (x1 + gb * f).astype(out_ref.dtype)
            cp = pltpu.make_async_copy(out_ref.at[r0:r1, :], out_hbm.at[r0:r1, :], sem_out.at[t])
            cp.start()
            cp_out.append(cp)
        for cp in cp_out:
            cp.wait()

    return kernel


def _run(A_x, A_wqkv, A_wo, B_x, B_w1, B_b1, B_w2, B_b2, c, w_mod, *, tq=256, ck=128, U=28, lag=4,
        tm=(512, 512, 512, 512), td=(512, 512, 512, 256, 256), early=1):
    del B_x
    B, S, D = A_x.shape
    F = B_w1.shape[1]
    assert (B, D) == (1, _D) and sum(tm) == S and sum(td) == S and U % 2 == 0 and 0 < lag <= S // ck // 2
    hbm = pl.BlockSpec(memory_space=pl.ANY)
    bf, u32, f32, V = jnp.bfloat16, jnp.uint32, jnp.float32, pltpu.VMEM
    out = pl.pallas_call(
        _make_kernel(S, F, tq, ck, U, lag, _offs(tm), _offs(td), early),
        in_specs=[hbm] * 9,
        out_specs=hbm,
        out_shape=jax.ShapeDtypeStruct((S, D), A_x.dtype),
        scratch_shapes=[
            V((S, D), bf), V((D, D), bf), V((D, D), bf), V((D, D), bf), V((D, D), bf),
            V((D, F), bf), V((F, D), bf), V((D, 2 * D), bf), V((D, 4 * D), bf), V((S, D), bf),
            V((S // 128, D // 2, 128), u32), V((4, S // 2, 128), u32),
            V((S // 128, D // 2, 128), u32), V((S // 128, D // 2, 128), u32),
            V((S, tq), f32), V((S, tq), f32), V((8, tq), f32), V((8, tq), f32),
            V((tq // 128, 64, 128), u32), V((tq // 128, 64, 128), u32),
            V((F,), bf), V((D,), bf), V((1, D), bf),
            pltpu.SemaphoreType.DMA((11,)), pltpu.SemaphoreType.DMA((len(tm),)),
            pltpu.SemaphoreType.DMA((len(td),)),
        ],
        compiler_params=pltpu.CompilerParams(vmem_limit_bytes=100 * 1024 * 1024),
    )(A_x.reshape(S, D), A_wqkv, A_wo, B_w1, B_b1, B_w2, B_b2, c, w_mod)
    return out.reshape(B, S, D)


@jax.jit
def pallas_adaLN_cond__mha_block__dense_activation_squared_relu__prompt_kernel(
    A_x: jax.Array,
    A_wqkv: jax.Array,
    A_wo: jax.Array,
    B_x: jax.Array,
    B_w1: jax.Array,
    B_b1: jax.Array,
    B_w2: jax.Array,
    B_b2: jax.Array,
    c: jax.Array,
    w_mod: jax.Array,
):
    return _run(A_x, A_wqkv, A_wo, B_x, B_w1, B_b1, B_w2, B_b2, c, w_mod)
```
